```python
import os as _os
_os.environ.setdefault("JAX_PLATFORMS", "cpu")
import jax
import jax.numpy as jnp

def _softmax(x, axis=-1):
    return jax.nn.softmax(x, axis=axis)
def _gelu(x):
    return jax.nn.gelu(x, approximate=True)
def _silu(x):
    return jax.nn.silu(x)
def _sigmoid(x):
    return jax.nn.sigmoid(x)
def _layernorm(x, axis=-1, eps=1e-5):
    m = jnp.mean(x, axis=axis, keepdims=True)
    v = jnp.var(x, axis=axis, keepdims=True)
    return (x - m) / jnp.sqrt(v + eps)
def _scatter_add(tgt, idx, src, axis=0):
    return tgt.at[idx].add(src)
def _segment_sum(src, seg, n):
    return jax.ops.segment_sum(src, seg, n)
class _Rng:
    def __init__(self, key):
        self._k = key
    def _next(self):
        self._k, sub = jax.random.split(self._k)
        return sub
    def normal(self, shape):
        return jax.random.normal(self._next(), shape, dtype=jnp.bfloat16)
    def randint(self, lo, hi, shape):
        return jax.random.randint(self._next(), shape, lo, hi, dtype=jnp.int32)
    def uniform(self, shape, lo=0.0, hi=1.0):
        return jax.random.uniform(self._next(), shape, jnp.bfloat16, lo, hi)
    def permutation(self, n):
        return jax.random.permutation(self._next(), n)


kernel_name = 'gated_mix__linear_attn_block__glu_gated_swiglu__prompt'

def setup_inputs():
    _rng = _Rng(jax.random.key(int.from_bytes(__import__("os").urandom(4), "little")))
    _w = (lambda a: (lambda t: t.astype(jnp.bfloat16) if jnp.issubdtype(t.dtype, jnp.floating) else t)(jnp.asarray(a)))
    def _A_setup():
        B, S, D = 1, 2048, 1024
        return {
            "x": _w((lambda *s: _rng.normal(s) * 0.05)(B, S, D)),
            "wqkv": _w((lambda *s: _rng.normal(s) * 0.8)(D, 3 * D)),
            "wo": _w((lambda *s: _rng.normal(s) * 0.05)(D, D)),
        }
    _A_in = _A_setup()

    def _B_setup():
        B, S, D, F = 1, 2048, 1024, 3584
        return {
            "x": _w((lambda *s: _rng.normal(s) * 0.05)(B, S, D)),
            "w1": _w((lambda *s: _rng.normal(s) * 1.6)(D, F) * (2.0 / D) ** 0.5),
            "w3": _w((lambda *s: _rng.normal(s) * 1.6)(D, F) * (2.0 / D) ** 0.5),
            "w2": _w((lambda *s: _rng.normal(s) * 1.6)(F, D) * (2.0 / F) ** 0.5),
        }
    _B_in = _B_setup()

    return {
        "A_x": _A_in["x"],
        "A_wqkv": _A_in["wqkv"],
        "A_wo": _A_in["wo"],
        "B_x": _B_in["x"],
        "B_w1": _B_in["w1"],
        "B_w3": _B_in["w3"],
        "B_w2": _B_in["w2"],
        "gate_w": _w((lambda *s: _rng.normal(s) * 0.05)(1024) * 16.0),
    }

def reference(A_x, A_wqkv, A_wo, B_x, B_w1, B_w3, B_w2, gate_w):
    def _A_ref(x, wqkv, wo):
        B, S, D = x.shape
        H = 32; Dh = D // H
        qkv = (lambda x, *d: x.transpose(*d))((x @ wqkv).reshape(B, S, 3, H, Dh), 2, 0, 3, 1, 4)
        q, k, v = qkv[0], qkv[1], qkv[2]
        phi = lambda t: jnp.where(t > 0, t + 1, jnp.exp(t)) + 1e-6
        pq, pk = phi(q), phi(k)
        kv = jnp.einsum("bhsd,bhse->bhde", pk, v)
        z = jnp.einsum("bhsd->bhd", pk)
        num = jnp.einsum("bhqd,bhde->bhqe", pq, kv)
        den = jnp.einsum("bhqd,bhd->bhq", pq, z)[..., None] + 1e-6
        o = num / den
        return (lambda x, *d: x.transpose(*d))(o, 0, 2, 1, 3).reshape(B, S, D) @ wo

    def _B_ref(x, w1, w3, w2):
        gate = jnp.einsum("bsd,df->bsf", x, w1)
        up = jnp.einsum("bsd,df->bsf", x, w3)
        h = _silu(gate) * up
        out = jnp.einsum("bsf,fd->bsd", h, w2)
        return out

    x = A_x
    g = _sigmoid((x * gate_w).sum(-1, keepdims=True))
    a = _A_ref(x, A_wqkv, A_wo)
    b = _B_ref(x, B_w1, B_w3, B_w2)
    return g * a + (1 - g) * b
```

```python
import jax
import jax.numpy as jnp
from jax import lax
import jax.experimental.pallas as pl
import jax.experimental.pallas.tpu as pltpu

_H = 32
_LANE = 128

_TM = 512
_TF = 512


def _phi(t):
    return jnp.where(t > 0, t + 1.0, jnp.exp(t)) + 1e-6


def _dot(a, b):
    return jnp.dot(a, b, preferred_element_type=jnp.float32)


def _make_kernel(S, D, F, tm, tf):
    dh = D // _H
    ng = D // _LANE
    nf = F // tf
    n_s = S // tm

    def kernel(x_ref, gw_ref, wqkv_hbm, wo_hbm, w1_hbm, w3_hbm, w2_hbm, o_ref,
               wq_s, wk_s, wv_s, wo_s, w1_s, w3_s, w2_s, kv_acc, z_acc, kvz_bf,
               sems):
        p = pl.program_id(0)
        i = pl.program_id(1)

        def weight_copies_early():
            return [
                pltpu.make_async_copy(wqkv_hbm.at[:, pl.ds(D, D)], wk_s, sems.at[0]),
                pltpu.make_async_copy(wqkv_hbm.at[:, pl.ds(2 * D, D)], wv_s, sems.at[1]),
            ]

        def weight_copies_late():
            cps = [
                pltpu.make_async_copy(wqkv_hbm.at[:, pl.ds(0, D)], wq_s, sems.at[2]),
                pltpu.make_async_copy(wo_hbm, wo_s, sems.at[3]),
            ]
            for f in range(nf):
                cps.append(pltpu.make_async_copy(
                    w1_hbm.at[:, pl.ds(f * tf, tf)], w1_s.at[f], sems.at[4 + 3 * f]))
                cps.append(pltpu.make_async_copy(
                    w3_hbm.at[:, pl.ds(f * tf, tf)], w3_s.at[f], sems.at[5 + 3 * f]))
                cps.append(pltpu.make_async_copy(
                    w2_hbm.at[pl.ds(f * tf, tf), :], w2_s.at[f], sems.at[6 + 3 * f]))
            return cps

        @pl.when(p == 0)
        def _phase0():
            @pl.when(i == 0)
            def _():
                for c in weight_copies_early():
                    c.start()
                for c in weight_copies_late():
                    c.start()
                kv_acc[...] = jnp.zeros_like(kv_acc)
                z_acc[...] = jnp.zeros_like(z_acc)
                for c in weight_copies_early():
                    c.wait()

            x = x_ref[...]
            k = _dot(x, wk_s[...])
            pk = _phi(k).astype(jnp.bfloat16)
            v = _dot(x, wv_s[...]).astype(jnp.bfloat16)
            z_acc[...] += jnp.sum(pk.astype(jnp.float32), axis=0, keepdims=True)
            for g in range(ng):
                sl = slice(g * _LANE, (g + 1) * _LANE)
                kv_acc[g] += lax.dot_general(
                    pk[:, sl], v[:, sl], (((0,), (0,)), ((), ())),
                    preferred_element_type=jnp.float32)

        @pl.when(p == 1)
        def _phase1():
            @pl.when(i == 0)
            def _():
                for c in weight_copies_late():
                    c.wait()
                r = lax.broadcasted_iota(jnp.int32, (_LANE, _LANE), 0) // dh
                c_ = lax.broadcasted_iota(jnp.int32, (_LANE, _LANE), 1) // dh
                same = r == c_
                z = z_acc[...]
                for g in range(ng):
                    sl = slice(g * _LANE, (g + 1) * _LANE)
                    zb = jnp.broadcast_to(z[:, sl], (_LANE, _LANE)).T
                    kvz_bf[g, :, :_LANE] = jnp.where(same, kv_acc[g], 0.0).astype(jnp.bfloat16)
                    kvz_bf[g, :, _LANE:] = jnp.where(same, zb, 0.0).astype(jnp.bfloat16)

            x = x_ref[...]
            gl = jnp.sum(x.astype(jnp.float32) * gw_ref[...].astype(jnp.float32),
                         axis=-1, keepdims=True)
            gate = jax.nn.sigmoid(gl)

            pq = _phi(_dot(x, wq_s[...])).astype(jnp.bfloat16)
            o_parts = []
            for g in range(ng):
                sl = slice(g * _LANE, (g + 1) * _LANE)
                nd = _dot(pq[:, sl], kvz_bf[g])
                o_parts.append((nd[:, :_LANE] / (nd[:, _LANE:] + 1e-6)).astype(jnp.bfloat16))
            o = jnp.concatenate(o_parts, axis=1)
            a = _dot(o, wo_s[...])

            b = None
            for f in range(nf):
                h1 = _dot(x, w1_s[f])
                h3 = _dot(x, w3_s[f])
                h = (jax.nn.silu(h1) * h3).astype(jnp.bfloat16)
                part = _dot(h, w2_s[f])
                b = part if b is None else b + part

            o_ref[...] = (gate * a + (1.0 - gate) * b).astype(o_ref.dtype)

    return kernel, n_s, nf, ng


@jax.jit
def pallas_gated_mix__linear_attn_block__glu_gated_swiglu__prompt_kernel(
    A_x: jax.Array,
    A_wqkv: jax.Array,
    A_wo: jax.Array,
    B_x: jax.Array,
    B_w1: jax.Array,
    B_w3: jax.Array,
    B_w2: jax.Array,
    gate_w: jax.Array,
):
    del B_x
    B, S, D = A_x.shape
    assert B == 1
    F = B_w1.shape[1]
    tm, tf = _TM, _TF
    kernel, n_s, nf, ng = _make_kernel(S, D, F, tm, tf)
    x2 = A_x.reshape(S, D)
    gw2 = gate_w.reshape(1, D)
    bf = jnp.bfloat16

    out = pl.pallas_call(
        kernel,
        grid=(2, n_s),
        in_specs=[
            pl.BlockSpec((tm, D), lambda p, i: (i, 0)),
            pl.BlockSpec((1, D), lambda p, i: (0, 0)),
            pl.BlockSpec(memory_space=pl.ANY),
            pl.BlockSpec(memory_space=pl.ANY),
            pl.BlockSpec(memory_space=pl.ANY),
            pl.BlockSpec(memory_space=pl.ANY),
            pl.BlockSpec(memory_space=pl.ANY),
        ],
        out_specs=pl.BlockSpec((tm, D), lambda p, i: (i * p, 0)),
        out_shape=jax.ShapeDtypeStruct((S, D), A_x.dtype),
        scratch_shapes=[
            pltpu.VMEM((D, D), bf),
            pltpu.VMEM((D, D), bf),
            pltpu.VMEM((D, D), bf),
            pltpu.VMEM((D, D), bf),
            pltpu.VMEM((nf, D, tf), bf),
            pltpu.VMEM((nf, D, tf), bf),
            pltpu.VMEM((nf, tf, D), bf),
            pltpu.VMEM((ng, _LANE, _LANE), jnp.float32),
            pltpu.VMEM((1, D), jnp.float32),
            pltpu.VMEM((ng, _LANE, 2 * _LANE), bf),
            pltpu.SemaphoreType.DMA((4 + 3 * nf,)),
        ],
        compiler_params=pltpu.CompilerParams(
            dimension_semantics=("arbitrary", "arbitrary"),
            vmem_limit_bytes=100 * 1024 * 1024,
        ),
    )(x2, gw2, A_wqkv, A_wo, B_w1, B_w3, B_w2)
    return out.reshape(B, S, D)
```

```python
import jax
import jax.numpy as jnp
from jax import lax
import jax.experimental.pallas as pl
import jax.experimental.pallas.tpu as pltpu

_H = 32
_LANE = 128

_TM = 256
_TF = 512
_NKC = 4


def _phi(t):
    return jnp.where(t > 0, t + 1.0, jnp.exp(t)) + 1e-6


def _dot(a, b):
    return jnp.dot(a, b, preferred_element_type=jnp.float32)


def _make_kernel(S, D, F, tm, tf, nkc):
    dh = D // _H
    ng = D // _LANE
    nf = F // tf
    n_s = S // tm
    kc = D // nkc
    bf = jnp.bfloat16

    SX = 0
    SK = SX + n_s
    SV = SK + nkc
    SQ = SV + nkc
    SO = SQ + 1
    SW = SO + 1
    SOUT = SW + 3 * nf
    n_sems = SOUT + 2

    def kernel(x_hbm, gw_ref, wqkv_hbm, wo_hbm, w1_hbm, w3_hbm, w2_hbm, out_hbm,
               x_s, wq_s, wk_s, wv_s, wo_s, w1_s, w3_s, w2_s, kv_acc, z_acc,
               kvz_bf, o_buf, sems):

        def x_copy(i):
            return pltpu.make_async_copy(
                x_hbm.at[pl.ds(i * tm, tm), :], x_s.at[i], sems.at[SX + i])

        def wk_copy(c):
            return pltpu.make_async_copy(
                wqkv_hbm.at[:, pl.ds(D + c * kc, kc)], wk_s.at[c], sems.at[SK + c])

        def wv_copy(c):
            return pltpu.make_async_copy(
                wqkv_hbm.at[:, pl.ds(2 * D + c * kc, kc)], wv_s.at[c], sems.at[SV + c])

        def late_copies():
            cps = [
                pltpu.make_async_copy(wqkv_hbm.at[:, pl.ds(0, D)], wq_s, sems.at[SQ]),
                pltpu.make_async_copy(wo_hbm, wo_s, sems.at[SO]),
            ]
            for f in range(nf):
                cps.append(pltpu.make_async_copy(
                    w1_hbm.at[:, pl.ds(f * tf, tf)], w1_s.at[f], sems.at[SW + 3 * f]))
                cps.append(pltpu.make_async_copy(
                    w3_hbm.at[:, pl.ds(f * tf, tf)], w3_s.at[f], sems.at[SW + 3 * f + 1]))
                cps.append(pltpu.make_async_copy(
                    w2_hbm.at[pl.ds(f * tf, tf), :], w2_s.at[f], sems.at[SW + 3 * f + 2]))
            return cps

        def out_copy(i, slot):
            return pltpu.make_async_copy(
                o_buf.at[slot], out_hbm.at[pl.ds(pl.multiple_of(i * tm, tm), tm), :],
                sems.at[SOUT + slot])

        def phase0_tile(i, first):
            if first:
                x_copy(0).wait()
            x = x_s[i]
            pks = []
            for c in range(nkc):
                if first:
                    wk_copy(c).wait()
                pks.append(_phi(_dot(x, wk_s[c])).astype(bf))
            if first:
                for j in range(1, n_s):
                    x_copy(j).start()
            vs = []
            for c in range(nkc):
                if first:
                    wv_copy(c).wait()
                vs.append(_dot(x, wv_s[c]).astype(bf))
            gpc = kc // _LANE
            for c in range(nkc):
                zc = jnp.sum(pks[c].astype(jnp.float32), axis=0, keepdims=True)
                if first:
                    z_acc[:, c * kc:(c + 1) * kc] = zc
                else:
                    z_acc[:, c * kc:(c + 1) * kc] += zc
                for gg in range(gpc):
                    g = c * gpc + gg
                    sl = slice(gg * _LANE, (gg + 1) * _LANE)
                    part = lax.dot_general(
                        pks[c][:, sl], vs[c][:, sl], (((0,), (0,)), ((), ())),
                        preferred_element_type=jnp.float32)
                    if first:
                        kv_acc[g] = part
                    else:
                        kv_acc[g] += part

        x_copy(0).start()
        for c in range(nkc):
            wk_copy(c).start()
        for c in range(nkc):
            wv_copy(c).start()

        phase0_tile(0, True)
        for cp in late_copies():
            cp.start()

        def p0_body(i, carry):
            x_copy_dyn = pltpu.make_async_copy(
                x_hbm.at[pl.ds(pl.multiple_of(i * tm, tm), tm), :], x_s.at[i],
                sems.at[SX + i])
            x_copy_dyn.wait()
            phase0_tile(i, False)
            return carry

        lax.fori_loop(1, n_s, p0_body, 0)

        r = lax.broadcasted_iota(jnp.int32, (_LANE, _LANE), 0) // dh
        c_ = lax.broadcasted_iota(jnp.int32, (_LANE, _LANE), 1) // dh
        same = r == c_
        z = z_acc[...]
        for g in range(ng):
            sl = slice(g * _LANE, (g + 1) * _LANE)
            zb = jnp.broadcast_to(z[:, sl], (_LANE, _LANE)).T
            kvz_bf[g, :, :_LANE] = jnp.where(same, kv_acc[g], 0.0).astype(bf)
            kvz_bf[g, :, _LANE:] = jnp.where(same, zb, 0.0).astype(bf)

        for cp in late_copies():
            cp.wait()

        gw = gw_ref[...].reshape(1, D).astype(jnp.float32)

        def p1_body(i, carry):
            slot = lax.rem(i, 2)
            x = x_s[i]
            gl = jnp.sum(x.astype(jnp.float32) * gw, axis=-1, keepdims=True)
            gate = jax.nn.sigmoid(gl)

            pq = _phi(_dot(x, wq_s[...])).astype(bf)
            o_parts = []
            for g in range(ng):
                sl = slice(g * _LANE, (g + 1) * _LANE)
                nd = _dot(pq[:, sl], kvz_bf[g])
                o_parts.append((nd[:, :_LANE] / (nd[:, _LANE:] + 1e-6)).astype(bf))
            o = jnp.concatenate(o_parts, axis=1)
            a = _dot(o, wo_s[...])

            b = None
            for f in range(nf):
                h1 = _dot(x, w1_s[f])
                h3 = _dot(x, w3_s[f])
                h = (jax.nn.silu(h1) * h3).astype(bf)
                part = _dot(h, w2_s[f])
                b = part if b is None else b + part

            res = (gate * a + (1.0 - gate) * b).astype(o_buf.dtype)

            @pl.when(i >= 2)
            def _():
                out_copy(i - 2, slot).wait()

            o_buf[slot] = res
            out_copy(i, slot).start()
            return carry

        lax.fori_loop(0, n_s, p1_body, 0)
        out_copy(n_s - 2, (n_s - 2) % 2).wait()
        out_copy(n_s - 1, (n_s - 1) % 2).wait()

    scratch = [
        pltpu.VMEM((n_s, tm, D), bf),
        pltpu.VMEM((D, D), bf),
        pltpu.VMEM((nkc, D, kc), bf),
        pltpu.VMEM((nkc, D, kc), bf),
        pltpu.VMEM((D, D), bf),
        pltpu.VMEM((nf, D, tf), bf),
        pltpu.VMEM((nf, D, tf), bf),
        pltpu.VMEM((nf, tf, D), bf),
        pltpu.VMEM((ng, _LANE, _LANE), jnp.float32),
        pltpu.VMEM((1, D), jnp.float32),
        pltpu.VMEM((ng, _LANE, 2 * _LANE), bf),
        pltpu.VMEM((2, tm, D), bf),
        pltpu.SemaphoreType.DMA((n_sems,)),
    ]
    return kernel, scratch


@jax.jit
def pallas_gated_mix__linear_attn_block__glu_gated_swiglu__prompt_kernel(
    A_x: jax.Array,
    A_wqkv: jax.Array,
    A_wo: jax.Array,
    B_x: jax.Array,
    B_w1: jax.Array,
    B_w3: jax.Array,
    B_w2: jax.Array,
    gate_w: jax.Array,
):
    del B_x
    B, S, D = A_x.shape
    assert B == 1
    F = B_w1.shape[1]
    kernel, scratch = _make_kernel(S, D, F, _TM, _TF, _NKC)
    x2 = A_x.reshape(S, D)

    hbm = pl.BlockSpec(memory_space=pl.ANY)
    out = pl.pallas_call(
        kernel,
        in_specs=[hbm, pl.BlockSpec(memory_space=pltpu.VMEM), hbm, hbm, hbm, hbm, hbm],
        out_specs=hbm,
        out_shape=jax.ShapeDtypeStruct((S, D), A_x.dtype),
        scratch_shapes=scratch,
        compiler_params=pltpu.CompilerParams(
            vmem_limit_bytes=100 * 1024 * 1024,
        ),
    )(x2, gate_w, A_wqkv, A_wo, B_w1, B_w3, B_w2)
    return out.reshape(B, S, D)
```

```python
import jax
import jax.numpy as jnp
from jax import lax
import jax.experimental.pallas as pl
import jax.experimental.pallas.tpu as pltpu

_H = 32
_LANE = 128

_TM = 256
_TF = 512
_NKC = 4


def _phi(t):
    return jnp.where(t > 0, t + 1.0, jnp.exp(t)) + 1e-6


def _dot(a, b):
    return jnp.dot(a, b, preferred_element_type=jnp.float32)


def _make_kernel(S, D, F, tm, tf, nkc):
    dh = D // _H
    ng = D // _LANE
    nf = F // tf
    n_s = S // tm
    kc = D // nkc
    gpc = kc // _LANE
    bf = jnp.bfloat16
    f32 = jnp.float32

    SX = 0
    SK = SX + n_s
    SV = SK + nkc
    SL = SV + nkc
    SOUT = SL + 1
    n_sems = SOUT + 2

    def kernel(x_hbm, gw_ref, wqkv_hbm, wo_hbm, w1_hbm, w3_hbm, w2_hbm, out_hbm,
               x_s, wq_s, wk_s, wv_s, wo_s, w1_s, w3_s, w2_s, kv_acc, z_acc,
               kvz_bf, o_buf, m_s, t_s, sems):

        def x_copy(i):
            return pltpu.make_async_copy(
                x_hbm.at[pl.ds(pl.multiple_of(i * tm, tm), tm), :], x_s.at[i],
                sems.at[SX + i])

        def wk_copy(c):
            return pltpu.make_async_copy(
                wqkv_hbm.at[:, pl.ds(D + c * kc, kc)], wk_s.at[c], sems.at[SK + c])

        def wv_copy(c):
            return pltpu.make_async_copy(
                wqkv_hbm.at[:, pl.ds(2 * D + c * kc, kc)], wv_s.at[c], sems.at[SV + c])

        def late_copies():
            cps = [
                pltpu.make_async_copy(wqkv_hbm.at[:, pl.ds(0, D)], wq_s, sems.at[SL]),
                pltpu.make_async_copy(wo_hbm, wo_s, sems.at[SL]),
            ]
            for f in range(nf):
                cps.append(pltpu.make_async_copy(
                    w1_hbm.at[:, pl.ds(f * tf, tf)], w1_s.at[f], sems.at[SL]))
                cps.append(pltpu.make_async_copy(
                    w3_hbm.at[:, pl.ds(f * tf, tf)], w3_s.at[f], sems.at[SL]))
                cps.append(pltpu.make_async_copy(
                    w2_hbm.at[pl.ds(f * tf, tf), :], w2_s.at[f], sems.at[SL]))
            return cps

        def out_copy(i, slot):
            return pltpu.make_async_copy(
                o_buf.at[slot], out_hbm.at[pl.ds(pl.multiple_of(i * tm, tm), tm), :],
                sems.at[SOUT + slot])

        x_copy(0).start()
        for c in range(nkc):
            wk_copy(c).start()
        for c in range(nkc):
            wv_copy(c).start()
        for j in range(1, n_s):
            x_copy(j).start()
        for cp in late_copies():
            cp.start()

        def phase0_tile(i, first):
            x_copy(i).wait()
            if not first:
                x = x_s[i]
            pks = []
            for c in range(nkc):
                if first:
                    wk_copy(c).wait()
                    x = x_s[i]
                pks.append(_phi(_dot(x, wk_s[c])).astype(bf))
            vs = []
            for c in range(nkc):
                if first:
                    wv_copy(c).wait()
                    x = x_s[i]
                vs.append(_dot(x, wv_s[c]).astype(bf))
            for c in range(nkc):
                zc = jnp.sum(pks[c].astype(f32), axis=0, keepdims=True)
                if first:
                    z_acc[:, c * kc:(c + 1) * kc] = zc
                else:
                    z_acc[:, c * kc:(c + 1) * kc] += zc
                for gg in range(gpc):
                    g = c * gpc + gg
                    sl = slice(gg * _LANE, (gg + 1) * _LANE)
                    part = lax.dot_general(
                        pks[c][:, sl], vs[c][:, sl], (((0,), (0,)), ((), ())),
                        preferred_element_type=f32)
                    if first:
                        kv_acc[g] = part
                    else:
                        kv_acc[g] += part

        phase0_tile(0, True)

        def p0_body(i, carry):
            phase0_tile(i, False)
            return carry

        lax.fori_loop(1, n_s, p0_body, 0)

        r = lax.broadcasted_iota(jnp.int32, (_LANE, _LANE), 0) // dh
        c_ = lax.broadcasted_iota(jnp.int32, (_LANE, _LANE), 1) // dh
        same_head = r == c_
        z = z_acc[...]
        for g in range(ng):
            sl = slice(g * _LANE, (g + 1) * _LANE)
            zb = jnp.broadcast_to(z[:, sl], (_LANE, _LANE)).T
            kvz_bf[g, :, :_LANE] = jnp.where(same_head, kv_acc[g], 0.0).astype(bf)
            kvz_bf[g, :, _LANE:] = jnp.where(same_head, zb, 0.0).astype(bf)

        for cp in late_copies():
            cp.wait()
        for g in range(ng):
            sl = slice(g * _LANE, (g + 1) * _LANE)
            m_s[sl, :] = _dot(kvz_bf[g, :, :_LANE], wo_s[sl, :]).astype(bf)

        gw = gw_ref[...].reshape(1, D).astype(f32)

        def p1_body(i, carry):
            slot = lax.rem(i, 2)

            @pl.when(i >= 2)
            def _():
                out_copy(i - 2, slot).wait()

            x = x_s[i]
            gl = jnp.sum(x.astype(f32) * gw, axis=-1, keepdims=True)
            gate = jax.nn.sigmoid(gl)

            pq = _phi(_dot(x, wq_s[...])).astype(bf)

            def den_group(g):
                sl = slice(g * _LANE, (g + 1) * _LANE)
                den = _dot(pq[:, sl], kvz_bf[g, :, _LANE:]) + 1e-6
                t_s[:, sl] = (pq[:, sl].astype(f32) / den).astype(bf)

            todo = list(range(ng))
            a = None
            b = None
            for f in range(nf):
                if todo:
                    den_group(todo.pop(0))
                h1 = _dot(x, w1_s[f])
                if todo:
                    den_group(todo.pop(0))
                h3 = _dot(x, w3_s[f])
                if todo:
                    den_group(todo.pop(0))
                elif a is None:
                    a = _dot(t_s[...], m_s[...])
                h = (jax.nn.silu(h1) * h3).astype(bf)
                part = _dot(h, w2_s[f])
                b = part if b is None else b + part
            while todo:
                den_group(todo.pop(0))
            if a is None:
                a = _dot(t_s[...], m_s[...])

            o_buf[slot] = (gate * a + (1.0 - gate) * b).astype(o_buf.dtype)
            out_copy(i, slot).start()
            return carry

        lax.fori_loop(0, n_s, p1_body, 0)
        out_copy(n_s - 2, (n_s - 2) % 2).wait()
        out_copy(n_s - 1, (n_s - 1) % 2).wait()

    scratch = [
        pltpu.VMEM((n_s, tm, D), bf),
        pltpu.VMEM((D, D), bf),
        pltpu.VMEM((nkc, D, kc), bf),
        pltpu.VMEM((nkc, D, kc), bf),
        pltpu.VMEM((D, D), bf),
        pltpu.VMEM((nf, D, tf), bf),
        pltpu.VMEM((nf, D, tf), bf),
        pltpu.VMEM((nf, tf, D), bf),
        pltpu.VMEM((ng, _LANE, _LANE), f32),
        pltpu.VMEM((1, D), f32),
        pltpu.VMEM((ng, _LANE, 2 * _LANE), bf),
        pltpu.VMEM((2, tm, D), bf),
        pltpu.VMEM((D, D), bf),
        pltpu.VMEM((tm, D), bf),
        pltpu.SemaphoreType.DMA((n_sems,)),
    ]
    return kernel, scratch


@jax.jit
def pallas_gated_mix__linear_attn_block__glu_gated_swiglu__prompt_kernel(
    A_x: jax.Array,
    A_wqkv: jax.Array,
    A_wo: jax.Array,
    B_x: jax.Array,
    B_w1: jax.Array,
    B_w3: jax.Array,
    B_w2: jax.Array,
    gate_w: jax.Array,
):
    del B_x
    B, S, D = A_x.shape
    assert B == 1
    F = B_w1.shape[1]
    assert S % _TM == 0 and S // _TM >= 2 and F % _TF == 0 and D % (_NKC * _LANE) == 0
    kernel, scratch = _make_kernel(S, D, F, _TM, _TF, _NKC)
    x2 = A_x.reshape(S, D)

    hbm = pl.BlockSpec(memory_space=pl.ANY)
    out = pl.pallas_call(
        kernel,
        in_specs=[hbm, pl.BlockSpec(memory_space=pltpu.VMEM), hbm, hbm, hbm, hbm, hbm],
        out_specs=hbm,
        out_shape=jax.ShapeDtypeStruct((S, D), A_x.dtype),
        scratch_shapes=scratch,
        compiler_params=pltpu.CompilerParams(
            vmem_limit_bytes=100 * 1024 * 1024,
        ),
    )(x2, gate_w, A_wqkv, A_wo, B_w1, B_w3, B_w2)
    return out.reshape(B, S, D)
```

```python
import jax
import jax.numpy as jnp
from jax import lax
import jax.experimental.pallas as pl
import jax.experimental.pallas.tpu as pltpu

_H = 32
_LANE = 128

_TM = 256
_TF = 512
_NKC = 4


def _phi(t):
    return jnp.where(t > 0, t + 1.0, jnp.exp(t)) + 1e-6


def _dot(a, b):
    return jnp.dot(a, b, preferred_element_type=jnp.float32)


def _make_kernel(S, D, F, tm, tf, nkc):
    dh = D // _H
    ng = D // _LANE
    nf = F // tf
    n_s = S // tm
    kc = D // nkc
    gpc = kc // _LANE
    bf = jnp.bfloat16
    f32 = jnp.float32

    SX = 0
    SK = SX + n_s
    SV = SK + nkc
    SL = SV + nkc
    SOUT = SL + 1
    n_sems = SOUT + 2

    def kernel(x_hbm, gw_hbm, wqkv_hbm, wo_hbm, w1_hbm, w3_hbm, w2_hbm, out_hbm,
               x_s, wq_s, wk_s, wv_s, wo_s, w1_s, w3_s, w2_s, kv_acc, z_acc,
               o_buf, m_s, t_s, gw_s, sems):

        def x_copy(i):
            return pltpu.make_async_copy(
                x_hbm.at[pl.ds(pl.multiple_of(i * tm, tm), tm), :], x_s.at[i],
                sems.at[SX + i])

        def wk_copy(c):
            return pltpu.make_async_copy(
                wqkv_hbm.at[:, pl.ds(D + c * kc, kc)], wk_s.at[c], sems.at[SK + c])

        def wv_copy(c):
            return pltpu.make_async_copy(
                wqkv_hbm.at[:, pl.ds(2 * D + c * kc, kc)], wv_s.at[c], sems.at[SV + c])

        def late_copies():
            cps = [
                pltpu.make_async_copy(wqkv_hbm.at[:, pl.ds(0, D)], wq_s, sems.at[SL]),
                pltpu.make_async_copy(wo_hbm, wo_s, sems.at[SL]),
                pltpu.make_async_copy(gw_hbm, gw_s, sems.at[SL]),
            ]
            for f in range(nf):
                cps.append(pltpu.make_async_copy(
                    w1_hbm.at[:, pl.ds(f * tf, tf)], w1_s.at[f], sems.at[SL]))
                cps.append(pltpu.make_async_copy(
                    w3_hbm.at[:, pl.ds(f * tf, tf)], w3_s.at[f], sems.at[SL]))
                cps.append(pltpu.make_async_copy(
                    w2_hbm.at[pl.ds(f * tf, tf), :], w2_s.at[f], sems.at[SL]))
            return cps

        def out_copy(i, slot):
            return pltpu.make_async_copy(
                o_buf.at[slot], out_hbm.at[pl.ds(pl.multiple_of(i * tm, tm), tm), :],
                sems.at[SOUT + slot])

        x_copy(0).start()
        for c in range(nkc):
            wk_copy(c).start()
        for c in range(nkc):
            wv_copy(c).start()
        for j in range(1, n_s):
            x_copy(j).start()
        for cp in late_copies():
            cp.start()

        def phase0_tile(i, first):
            x_copy(i).wait()
            if not first:
                x = x_s[i]
            pks = []
            for c in range(nkc):
                if first:
                    wk_copy(c).wait()
                    x = x_s[i]
                pks.append(_phi(_dot(x, wk_s[c])).astype(bf))
            vs = []
            for c in range(nkc):
                if first:
                    wv_copy(c).wait()
                    x = x_s[i]
                vs.append(_dot(x, wv_s[c]).astype(bf))
            for c in range(nkc):
                zc = jnp.sum(pks[c].astype(f32), axis=0, keepdims=True)
                if first:
                    z_acc[:, c * kc:(c + 1) * kc] = zc
                else:
                    z_acc[:, c * kc:(c + 1) * kc] += zc
                for gg in range(gpc):
                    g = c * gpc + gg
                    sl = slice(gg * _LANE, (gg + 1) * _LANE)
                    part = lax.dot_general(
                        pks[c][:, sl], vs[c][:, sl], (((0,), (0,)), ((), ())),
                        preferred_element_type=f32)
                    if first:
                        kv_acc[g] = part
                    else:
                        kv_acc[g] += part

        phase0_tile(0, True)

        def p0_body(i, carry):
            phase0_tile(i, False)
            return carry

        lax.fori_loop(1, n_s, p0_body, 0)

        r = lax.broadcasted_iota(jnp.int32, (_LANE, _LANE), 0) // dh
        c_ = lax.broadcasted_iota(jnp.int32, (_LANE, _LANE), 1) // dh
        same_head = r == c_
        z = z_acc[...]
        for cp in late_copies():
            cp.wait()
        for g in range(ng):
            sl = slice(g * _LANE, (g + 1) * _LANE)
            kv_bd = jnp.where(same_head, kv_acc[g], 0.0).astype(bf)
            m_s[sl, :] = _dot(kv_bd, wo_s[sl, :]).astype(bf)

        gw = gw_s[...].reshape(1, D).astype(f32)

        def p1_body(i, carry):
            slot = lax.rem(i, 2)

            @pl.when(i >= 2)
            def _():
                out_copy(i - 2, slot).wait()

            x = x_s[i]
            gl = jnp.sum(x.astype(f32) * gw, axis=-1, keepdims=True)
            gate = jax.nn.sigmoid(gl)

            pq = _phi(_dot(x, wq_s[...])).astype(bf)
            lane = lax.broadcasted_iota(jnp.int32, (tm, _LANE), 1) % dh

            def den_group(g):
                sl = slice(g * _LANE, (g + 1) * _LANE)
                pqf = pq[:, sl].astype(f32)
                sacc = pqf * z[:, sl]
                k = 1
                while k < dh:
                    r1 = pltpu.roll(sacc, _LANE - k, 1)
                    r2 = pltpu.roll(sacc, dh - k, 1)
                    sacc = sacc + jnp.where(lane < dh - k, r1, r2)
                    k *= 2
                t_s[:, sl] = (pqf / (sacc + 1e-6)).astype(bf)

            todo = list(range(ng))
            a = None
            b = None
            for f in range(nf):
                if todo:
                    den_group(todo.pop(0))
                h1 = _dot(x, w1_s[f])
                if todo:
                    den_group(todo.pop(0))
                h3 = _dot(x, w3_s[f])
                if todo:
                    den_group(todo.pop(0))
                elif a is None:
                    a = _dot(t_s[...], m_s[...])
                h = (jax.nn.silu(h1) * h3).astype(bf)
                part = _dot(h, w2_s[f])
                b = part if b is None else b + part
            while todo:
                den_group(todo.pop(0))
            if a is None:
                a = _dot(t_s[...], m_s[...])

            o_buf[slot] = (gate * a + (1.0 - gate) * b).astype(o_buf.dtype)
            out_copy(i, slot).start()
            return carry

        lax.fori_loop(0, n_s, p1_body, 0)
        out_copy(n_s - 2, (n_s - 2) % 2).wait()
        out_copy(n_s - 1, (n_s - 1) % 2).wait()

    scratch = [
        pltpu.VMEM((n_s, tm, D), bf),
        pltpu.VMEM((D, D), bf),
        pltpu.VMEM((nkc, D, kc), bf),
        pltpu.VMEM((nkc, D, kc), bf),
        pltpu.VMEM((D, D), bf),
        pltpu.VMEM((nf, D, tf), bf),
        pltpu.VMEM((nf, D, tf), bf),
        pltpu.VMEM((nf, tf, D), bf),
        pltpu.VMEM((ng, _LANE, _LANE), f32),
        pltpu.VMEM((1, D), f32),
        pltpu.VMEM((2, tm, D), bf),
        pltpu.VMEM((D, D), bf),
        pltpu.VMEM((tm, D), bf),
        pltpu.VMEM((D,), bf),
        pltpu.SemaphoreType.DMA((n_sems,)),
    ]
    return kernel, scratch


@jax.jit
def pallas_gated_mix__linear_attn_block__glu_gated_swiglu__prompt_kernel(
    A_x: jax.Array,
    A_wqkv: jax.Array,
    A_wo: jax.Array,
    B_x: jax.Array,
    B_w1: jax.Array,
    B_w3: jax.Array,
    B_w2: jax.Array,
    gate_w: jax.Array,
):
    del B_x
    B, S, D = A_x.shape
    assert B == 1
    F = B_w1.shape[1]
    assert S % _TM == 0 and S // _TM >= 2 and F % _TF == 0 and D % (_NKC * _LANE) == 0
    kernel, scratch = _make_kernel(S, D, F, _TM, _TF, _NKC)
    x2 = A_x.reshape(S, D)

    hbm = pl.BlockSpec(memory_space=pl.ANY)
    out = pl.pallas_call(
        kernel,
        in_specs=[hbm] * 7,
        out_specs=hbm,
        out_shape=jax.ShapeDtypeStruct((S, D), A_x.dtype),
        scratch_shapes=scratch,
        compiler_params=pltpu.CompilerParams(
            vmem_limit_bytes=100 * 1024 * 1024,
        ),
    )(x2, gate_w, A_wqkv, A_wo, B_w1, B_w3, B_w2)
    return out.reshape(B, S, D)
```
